```python
import jax
import jax.numpy as jnp

def _softmax(x, axis=-1):
    return jax.nn.softmax(x, axis=axis)
def _gelu(x):
    return jax.nn.gelu(x, approximate=True)
def _silu(x):
    return jax.nn.silu(x)
def _sigmoid(x):
    return jax.nn.sigmoid(x)
def _layernorm(x, axis=-1, eps=1e-5):
    m = jnp.mean(x, axis=axis, keepdims=True)
    v = jnp.var(x, axis=axis, keepdims=True)
    return (x - m) / jnp.sqrt(v + eps)
def _scatter_add(tgt, idx, src, axis=0):
    return tgt.at[idx].add(src)
def _segment_sum(src, seg, n):
    return jax.ops.segment_sum(src, seg, n)
class _Rng:
    def __init__(self, key):
        self._k = key
    def _next(self):
        self._k, sub = jax.random.split(self._k)
        return sub
    def normal(self, shape):
        return jax.random.normal(self._next(), shape, dtype=jnp.bfloat16)
    def randint(self, lo, hi, shape):
        return jax.random.randint(self._next(), shape, lo, hi, dtype=jnp.int32)
    def uniform(self, shape, lo=0.0, hi=1.0):
        return jax.random.uniform(self._next(), shape, jnp.bfloat16, lo, hi)
    def permutation(self, n):
        return jax.random.permutation(self._next(), n)


kernel_name = 'recurrent_scan__sliding_block_cached__glu_gated_swiglu__decode'

def setup_inputs():
    _rng = _Rng(jax.random.key(int.from_bytes(__import__("os").urandom(4), "little")))
    _w = (lambda a: (lambda t: t.astype(jnp.bfloat16) if jnp.issubdtype(t.dtype, jnp.floating) else t)(jnp.asarray(a)))
    def _A_setup():
        B, Sq, D = 1, 1, 640
        Hq, Hkv, Sk, Dh = 32, 32, 32768, 192
        assert Hq % Hkv == 0, (Hq, Hkv)
        return {
            "x": _w((lambda *s: _rng.normal(s) * 0.05)(B, Sq, D)),
            "k_cache": _w((lambda *s: _rng.normal(s) * 0.05)(B, Hkv, Sk, Dh)),
            "v_cache": _w((lambda *s: _rng.normal(s) * 0.05)(B, Hkv, Sk, Dh)),
            "wq": _w((lambda *s: _rng.normal(s) * 0.05)(D, Hq * Dh) * (D ** -0.5)),
            "wo": _w((lambda *s: _rng.normal(s) * 0.05)(Hq * Dh, D) * ((Hq * Dh) ** -0.5)),
        }
    _A_in = _A_setup()

    def _B_setup():
        B, S, D, F = 1, 1, 640, 1536
        return {
            "x": _w((lambda *s: _rng.normal(s) * 0.05)(B, S, D)),
            "w1": _w((lambda *s: _rng.normal(s) * 0.05)(D, F) * (2.0 / D) ** 0.5),
            "w3": _w((lambda *s: _rng.normal(s) * 0.05)(D, F) * (2.0 / D) ** 0.5),
            "w2": _w((lambda *s: _rng.normal(s) * 0.05)(F, D) * (2.0 / F) ** 0.5),
        }
    _B_in = _B_setup()

    return {
        "A_x": _A_in["x"],
        "A_k_cache": _A_in["k_cache"],
        "A_v_cache": _A_in["v_cache"],
        "A_wq": _A_in["wq"],
        "A_wo": _A_in["wo"],
        "B_x": _B_in["x"],
        "B_w1": _B_in["w1"],
        "B_w3": _B_in["w3"],
        "B_w2": _B_in["w2"],
    }

def reference(A_x, A_k_cache, A_v_cache, A_wq, A_wo, B_x, B_w1, B_w3, B_w2):
    def _A_ref(x, k_cache, v_cache, wq, wo):
        B, Sq, D = x.shape
        Hq, Dh = 32, 192
        Hkv, Sk = k_cache.shape[1], k_cache.shape[2]
        W = min(4096, max(256, Sk // 4))
        rep = Hq // Hkv
        q = (lambda x, *d: x.transpose(*d))((x @ wq).reshape(B, Sq, Hq, Dh), 0, 2, 1, 3)
        k = jnp.repeat(k_cache[:, :, Sk - W:, :], rep, axis=1)
        v = jnp.repeat(v_cache[:, :, Sk - W:, :], rep, axis=1)
        scores = jnp.einsum("bhqd,bhkd->bhqk", q, k) * (Dh ** -0.5)
        p = _softmax(scores, axis=-1)
        o = jnp.einsum("bhqk,bhkd->bhqd", p, v)
        return (lambda x, *d: x.transpose(*d))(o, 0, 2, 1, 3).reshape(B, Sq, Hq * Dh) @ wo

    def _B_ref(x, w1, w3, w2):
        gate = jnp.einsum("bsd,df->bsf", x, w1)
        up = jnp.einsum("bsd,df->bsf", x, w3)
        h = _silu(gate) * up
        out = jnp.einsum("bsf,fd->bsd", h, w2)
        return out

    x = A_x
    xn = _layernorm(x, axis=-1)
    s = _A_ref(xn, A_k_cache, A_v_cache, A_wq, A_wo)
    g = _silu(_B_ref(xn, B_w1, B_w3, B_w2))
    return x + s * g
```

```python
import functools

import jax
import jax.numpy as jnp
from jax import lax
import jax.experimental.pallas as pl
import jax.experimental.pallas.tpu as pltpu

HQ, DH = 32, 192
EPS = 1e-5

LOOKAHEAD = 8
GW = 1024
KV_CR = 16
QG, WQ_CR = 1024, 16
FG, FF_CR = 512, 32
WO_HB, WO_CR = 2, 32
WQ_LOOKAHEAD = 3
M = 8


def _kernel(x_hbm, k_hbm, v_hbm, wq_hbm, wo_hbm, w1_hbm, w3_hbm, w2_hbm, out_ref,
            x_v, wq_v, w1_v, w3_v, w2_v, wo_v, kv_v, qf_v, q_v, o_v,
            x_sem, wq_sem, ff_sem, wo_sem, kv_sem, *, window):
    f32, bf16 = jnp.float32, jnp.bfloat16
    n_heads, _, sk = k_hbm.shape
    d_model = wq_hbm.shape[0]
    ng = window // GW
    pb = 2 * ng
    nqg, nfg, nwo = wq_v.shape[0], w1_v.shape[0], wo_v.shape[0]
    wo_rows = WO_HB * DH

    def start_rows(src, dst, sem, nrows, cr):
        def body(i, c):
            for p in range(2):
                r = pl.multiple_of((2 * i + p) * cr, cr)
                pltpu.make_async_copy(src.at[pl.ds(r, cr)], dst.at[pl.ds(r, cr)], sem).start(priority=p)
            return c
        lax.fori_loop(0, nrows // (2 * cr), body, 0)

    def wait_all(dst, sem):
        pltpu.make_async_copy(dst, dst, sem).wait()

    def start_wq(g):
        c = pl.multiple_of(g * QG, QG)
        start_rows(wq_hbm.at[:, pl.ds(c, QG)], wq_v.at[g], wq_sem.at[g], d_model, WQ_CR)

    def start_ff(g):
        c = pl.multiple_of(g * FG, FG)
        start_rows(w1_hbm.at[:, pl.ds(c, FG)], w1_v.at[g], ff_sem.at[g], d_model, FF_CR)
        start_rows(w3_hbm.at[:, pl.ds(c, FG)], w3_v.at[g], ff_sem.at[g], d_model, FF_CR)
        start_rows(w2_hbm.at[pl.ds(c, FG)], w2_v.at[g], ff_sem.at[g], FG, WO_CR)

    def wait_ff(g):
        wait_all(w1_v.at[g], ff_sem.at[g])
        wait_all(w3_v.at[g], ff_sem.at[g])
        wait_all(w2_v.at[g], ff_sem.at[g])

    def start_wo(j):
        r = pl.multiple_of(j * wo_rows, wo_rows)
        start_rows(wo_hbm.at[pl.ds(r, wo_rows)], wo_v.at[j], wo_sem.at[j], wo_rows, WO_CR)

    def start_kv(h, r):
        src = k_hbm if r < ng else v_hbm
        c = sk - window + (r % ng) * GW
        slot = (h % 2) * pb + r
        for i in range(DH // KV_CR):
            pltpu.make_async_copy(src.at[h, pl.ds(i * KV_CR, KV_CR), pl.ds(c, GW)],
                                  kv_v.at[slot, pl.ds(i * KV_CR, KV_CR)],
                                  kv_sem.at[slot]).start(priority=i % 2)

    for g in range(WQ_LOOKAHEAD):
        start_wq(g)
    cpx = pltpu.make_async_copy(x_hbm, x_v, x_sem)
    cpx.start()
    cpx.wait()
    x = x_v[0].astype(f32)
    xc = x - jnp.mean(x, axis=-1, keepdims=True)
    var = jnp.mean(xc * xc, axis=-1, keepdims=True)
    xn = jnp.broadcast_to(xc / jnp.sqrt(var + EPS), (M, d_model)).astype(bf16)

    def q_step(g, c):
        wait_all(wq_v.at[g], wq_sem.at[g])

        @pl.when(g + WQ_LOOKAHEAD < nqg)
        def _():
            start_wq(g + WQ_LOOKAHEAD)

        @pl.when(g + WQ_LOOKAHEAD >= nqg)
        def _():
            start_ff(g + WQ_LOOKAHEAD - nqg)

        qf_v[g] = jnp.dot(xn, wq_v[g], preferred_element_type=f32)
        return c
    lax.fori_loop(0, nqg, q_step, 0)

    per = -(-LOOKAHEAD // nfg)

    def ff_step(g, ff):
        wait_ff(g)
        for gg in range(nfg):
            @pl.when(g == gg)
            def _():
                for b in range(gg * per, min(LOOKAHEAD, (gg + 1) * per)):
                    start_kv(b // pb, b % pb)
        gate = jnp.dot(xn, w1_v[g], preferred_element_type=f32)
        up = jnp.dot(xn, w3_v[g], preferred_element_type=f32)
        hid = (gate * jax.nn.sigmoid(gate) * up).astype(bf16)
        return ff + jnp.dot(hid, w2_v[g], preferred_element_type=f32)
    ff = lax.fori_loop(0, nfg, ff_step, jnp.zeros((M, d_model), f32))
    gact = ff * jax.nn.sigmoid(ff)

    for h in range(n_heads):
        lo, hi = h * DH, (h + 1) * DH
        g0, g1 = lo // QG, (hi - 1) // QG
        if g0 == g1:
            q_v[h] = qf_v[g0, :, lo - g0 * QG:hi - g0 * QG]
        else:
            q_v[h] = jnp.concatenate([qf_v[g0, :, lo - g0 * QG:], qf_v[g1, :, :hi - g1 * QG]], axis=-1)

    scale = DH ** -0.5

    def head(h, c):
        base = (h % 2) * pb

        def advance(r):
            wait_all(kv_v.at[base + r], kv_sem.at[base + r])
            dh, rr = divmod(r + LOOKAHEAD, pb)

            @pl.when(h + dh < n_heads)
            def _():
                start_kv(h + dh, rr)

            @pl.when(h + dh >= n_heads)
            def _():
                start_wo((h + dh - n_heads) * pb + rr)

        qh = q_v[h].astype(bf16)
        s = []
        for r in range(ng):
            advance(r)
            s.append(jnp.dot(qh, kv_v[base + r], preferred_element_type=f32) * scale)
        m = jnp.max(functools.reduce(jnp.maximum, s), axis=-1, keepdims=True)
        p = [jnp.exp(si - m) for si in s]
        denom = jnp.sum(functools.reduce(jnp.add, p), axis=-1, keepdims=True)
        acc = jnp.zeros((M, DH), f32)
        for r in range(ng):
            advance(ng + r)
            acc = acc + lax.dot_general(p[r].astype(bf16), kv_v[base + ng + r], (((1,), (1,)), ((), ())),
                                        preferred_element_type=f32)
        o_v[h] = acc / denom
        return c
    lax.fori_loop(0, n_heads, head, 0)

    def wo_step(j, s):
        wait_all(wo_v.at[j], wo_sem.at[j])

        @pl.when(j + LOOKAHEAD < nwo)
        def _():
            start_wo(j + LOOKAHEAD)

        for t in range(WO_HB):
            s = s + jnp.dot(o_v[j * WO_HB + t].astype(bf16), wo_v[j, t * DH:(t + 1) * DH, :],
                            preferred_element_type=f32)
        return s
    s = lax.fori_loop(0, nwo, wo_step, jnp.zeros((M, d_model), f32))
    out_ref[0] = (x + s[0:1] * gact[0:1]).astype(out_ref.dtype)


@jax.jit
def pallas_recurrent_scan__sliding_block_cached__glu_gated_swiglu__decode_kernel(
    A_x: jax.Array,
    A_k_cache: jax.Array,
    A_v_cache: jax.Array,
    A_wq: jax.Array,
    A_wo: jax.Array,
    B_x: jax.Array,
    B_w1: jax.Array,
    B_w3: jax.Array,
    B_w2: jax.Array,
):
    del B_x
    d_model = A_x.shape[-1]
    _, hkv, sk, dh = A_k_cache.shape
    d_ff = B_w1.shape[1]
    window = min(4096, max(256, sk // 4))
    assert A_x.shape[:2] == (1, 1) and (hkv, dh) == (HQ, DH)
    assert window % GW == 0 and (HQ * DH) % QG == 0 and d_ff // FG == WQ_LOOKAHEAD
    nqg, nfg, nwo = HQ * DH // QG, d_ff // FG, HQ // WO_HB
    n_slots = 4 * (window // GW)
    bf16, f32 = jnp.bfloat16, jnp.float32

    kt = jnp.swapaxes(A_k_cache, 2, 3).reshape(hkv, dh, sk)
    vt = jnp.swapaxes(A_v_cache, 2, 3).reshape(hkv, dh, sk)

    hbm = pl.BlockSpec(memory_space=pltpu.HBM)
    return pl.pallas_call(
        functools.partial(_kernel, window=window),
        in_specs=[hbm] * 8,
        out_specs=pl.BlockSpec(memory_space=pltpu.VMEM),
        out_shape=jax.ShapeDtypeStruct(A_x.shape, A_x.dtype),
        scratch_shapes=[
            pltpu.VMEM((1, 1, d_model), bf16),
            pltpu.VMEM((nqg, d_model, QG), bf16),
            pltpu.VMEM((nfg, d_model, FG), bf16),
            pltpu.VMEM((nfg, d_model, FG), bf16),
            pltpu.VMEM((nfg, FG, d_model), bf16),
            pltpu.VMEM((nwo, WO_HB * DH, d_model), bf16),
            pltpu.VMEM((n_slots, DH, GW), bf16),
            pltpu.VMEM((nqg, M, QG), f32),
            pltpu.VMEM((HQ, M, DH), f32),
            pltpu.VMEM((HQ, M, DH), f32),
            pltpu.SemaphoreType.DMA(()),
            pltpu.SemaphoreType.DMA((nqg,)),
            pltpu.SemaphoreType.DMA((nfg,)),
            pltpu.SemaphoreType.DMA((nwo,)),
            pltpu.SemaphoreType.DMA((n_slots,)),
        ],
        compiler_params=pltpu.CompilerParams(vmem_limit_bytes=64 * 1024 * 1024),
    )(A_x, kt, vt, A_wq, A_wo, B_w1, B_w3, B_w2)
```

```python
import functools

import jax
import jax.numpy as jnp
from jax import lax
import jax.experimental.pallas as pl
import jax.experimental.pallas.tpu as pltpu

HQ, DH = 32, 192
EPS = 1e-5
M = 8
RG = 8

LOOKAHEAD = 8
KV_COLS, KV_ROWS = 1024, 16
WQ_SPLIT, WQ_COLS = 10, 1024
W13_SPLIT, W2_SPLIT, WO_SPLIT = 4, 3, 8


def _stream(x_hbm, k_hbm, v_hbm, wq_hbm, wo_hbm, w1_hbm, w3_hbm, w2_hbm, out_hbm,
            x_v, wq_v, w1_v, w3_v, w2_v, wo_v, kv_v, qf_v, q_v, o_v, io_sem, sems, *, window):
    f32, bf16 = jnp.float32, jnp.bfloat16
    ds = pl.ds
    n_heads, _, sk = k_hbm.shape
    d_model, d_ff = x_v.shape[-1], w1_v.shape[-1]
    ng = window // KV_COLS
    per_head = 2 * ng
    groups = n_heads // WO_SPLIT

    def batches(copies, n):
        return [copies[i:i + n] for i in range(0, len(copies), n)]

    def same_place(src, dst, *idx):
        return src.at[idx], dst.at[idx]

    pre, q_ready = [], {}
    for g in range(wq_v.shape[0]):
        pre += batches([(wq_hbm.at[ds(a, 2), ds(r, RG), ds(g * WQ_COLS, WQ_COLS)], wq_v.at[g, ds(a, 2), ds(r, RG)])
                        for r in range(0, wq_v.shape[2], RG) for a in range(0, WQ_SPLIT, 2)], WQ_SPLIT)
        q_ready[len(pre) - 1] = g
    ffn = [same_place(src, dst, ds(a, 2), ds(r, RG))
           for r in range(0, w1_v.shape[1], RG) for a in range(0, W13_SPLIT, 2)
           for src, dst in ((w1_hbm, w1_v), (w3_hbm, w3_v))]
    half = w2_v.shape[1] // 2
    ffn += [same_place(w2_hbm, w2_v, slice(None), ds(r + off, RG)) for r in range(0, half, RG) for off in (0, half)]
    pre += batches(ffn, 12)

    post, wo_ready = [], {}
    for j in range(groups):
        for lo, hi in ((0, 128), (128, DH)):
            post += batches([(wo_hbm.at[ds(a, 4), ds(j * DH + r, RG)], wo_v.at[ds(a, 4), j, ds(r, RG)])
                             for r in range(lo, hi, RG) for a in range(0, WO_SPLIT, 4)], 16)
            wo_ready[len(post) - 1] = (j, lo, hi)
    assert per_head == LOOKAHEAD and len(pre) >= LOOKAHEAD and len(post) >= LOOKAHEAD

    def sem(n):
        return sems.at[n % LOOKAHEAD]

    def start(copies, n):
        for i, (src, dst) in enumerate(copies):
            pltpu.make_async_copy(src, dst, sem(n)).start(priority=i % 2)

    def wait(copies, n):
        for src, dst in copies:
            pltpu.make_async_copy(src, dst, sem(n)).wait()

    def kv_slot(h, r):
        return (h % 2) * per_head + r

    def start_kv(h, r):
        src = k_hbm if r < ng else v_hbm
        col = sk - window + (r % ng) * KV_COLS
        start([(src.at[h, ds(i, KV_ROWS), ds(col, KV_COLS)], kv_v.at[kv_slot(h, r), ds(i, KV_ROWS)])
               for i in range(0, DH, KV_ROWS)], len(pre) + r)

    start(pre[0], 0)
    x_copy = pltpu.make_async_copy(x_hbm, x_v, io_sem)
    x_copy.start()
    for n in range(1, LOOKAHEAD):
        start(pre[n], n)
    x_copy.wait()
    x = x_v[0].astype(f32)
    xc = x - jnp.mean(x, axis=-1, keepdims=True)
    var = jnp.mean(xc * xc, axis=-1, keepdims=True)
    xn = jnp.broadcast_to(xc / jnp.sqrt(var + EPS), (M, d_model)).astype(bf16)

    for n, copies in enumerate(pre):
        wait(copies, n)
        if n + LOOKAHEAD < len(pre):
            start(pre[n + LOOKAHEAD], n + LOOKAHEAD)
        else:
            start_kv(0, n + LOOKAHEAD - len(pre))
        if n in q_ready:
            g = q_ready[n]
            qf_v[g] = jnp.dot(xn, wq_v[g].reshape(d_model, WQ_COLS), preferred_element_type=f32)
    gate = jnp.dot(xn, w1_v[...].reshape(d_model, d_ff), preferred_element_type=f32)
    up = jnp.dot(xn, w3_v[...].reshape(d_model, d_ff), preferred_element_type=f32)
    hidden = (gate * jax.nn.sigmoid(gate) * up).astype(bf16)
    ffn_out = jnp.dot(hidden, w2_v[...].reshape(d_ff, d_model), preferred_element_type=f32)
    ffn_gate = ffn_out * jax.nn.sigmoid(ffn_out)

    for h in range(n_heads):
        lo, hi = h * DH, (h + 1) * DH
        g0, g1 = lo // WQ_COLS, (hi - 1) // WQ_COLS
        if g0 == g1:
            q_v[h] = qf_v[g0, :, lo - g0 * WQ_COLS:hi - g0 * WQ_COLS]
        else:
            q_v[h] = jnp.concatenate([qf_v[g0, :, lo - g0 * WQ_COLS:], qf_v[g1, :, :hi - g1 * WQ_COLS]], axis=-1)

    scale = DH ** -0.5

    def head(h, carry):
        def next_tile(r):
            tile = kv_v.at[kv_slot(h, r)]
            wait([(tile, tile)], len(pre) + r)
            pl.when(h + 1 < n_heads)(lambda: start_kv(h + 1, r))
            pl.when(h + 1 == n_heads)(lambda: start(post[r], len(pre) + r))
            return tile[...]

        q = q_v[h].astype(bf16)
        s = [jnp.dot(q, next_tile(r), preferred_element_type=f32) * scale for r in range(ng)]
        m = jnp.max(functools.reduce(jnp.maximum, s), axis=-1, keepdims=True)
        p = [jnp.exp(si - m) for si in s]
        denom = jnp.sum(functools.reduce(jnp.add, p), axis=-1, keepdims=True)
        acc = jnp.zeros((M, DH), f32)
        for r in range(ng):
            acc = acc + lax.dot_general(p[r].astype(bf16), next_tile(ng + r), (((1,), (1,)), ((), ())),
                                        preferred_element_type=f32)
        o_v[h] = acc / denom
        return carry
    lax.fori_loop(0, n_heads, head, 0)

    y = jnp.zeros((M, d_model), f32)
    for n, copies in enumerate(post):
        if n in wo_ready:
            j, lo, hi = wo_ready[n]
            o = jnp.concatenate([o_v[a * groups + j, :, lo:hi] for a in range(WO_SPLIT)], axis=-1).astype(bf16)
        wait(copies, len(pre) + n)
        if n + LOOKAHEAD < len(post):
            start(post[n + LOOKAHEAD], len(pre) + n + LOOKAHEAD)
        if n in wo_ready:
            w = wo_v[:, j, lo:hi, :].reshape(WO_SPLIT * (hi - lo), d_model)
            y = y + jnp.dot(o, w, preferred_element_type=f32)

    x_v[0] = (x + y[0:1] * ffn_gate[0:1]).astype(x_v.dtype)
    pltpu.make_async_copy(x_v, out_hbm, io_sem).start()


def _kernel(*refs, window):
    out_hbm, x_v, io_sem = refs[8], refs[9], refs[-1]
    pl.run_scoped(functools.partial(_stream, *refs, window=window), pltpu.SemaphoreType.DMA((LOOKAHEAD,)))
    pltpu.make_async_copy(x_v, out_hbm, io_sem).wait()


@jax.jit
def pallas_recurrent_scan__sliding_block_cached__glu_gated_swiglu__decode_kernel(
    A_x: jax.Array,
    A_k_cache: jax.Array,
    A_v_cache: jax.Array,
    A_wq: jax.Array,
    A_wo: jax.Array,
    B_x: jax.Array,
    B_w1: jax.Array,
    B_w3: jax.Array,
    B_w2: jax.Array,
):
    del B_x
    d_model = A_x.shape[-1]
    _, hkv, sk, dh = A_k_cache.shape
    d_ff = B_w1.shape[1]
    window = min(4096, max(256, sk // 4))
    assert A_x.shape[:2] == (1, 1) and (hkv, dh) == (HQ, DH) and window % KV_COLS == 0
    bf16, f32 = jnp.bfloat16, jnp.float32

    kt = jnp.swapaxes(A_k_cache, 2, 3).reshape(hkv, dh, sk)
    vt = jnp.swapaxes(A_v_cache, 2, 3).reshape(hkv, dh, sk)
    wq = A_wq.reshape(WQ_SPLIT, d_model // WQ_SPLIT, HQ * DH)
    wo = A_wo.reshape(WO_SPLIT, HQ * DH // WO_SPLIT, d_model)
    w1 = B_w1.reshape(W13_SPLIT, d_model // W13_SPLIT, d_ff)
    w3 = B_w3.reshape(W13_SPLIT, d_model // W13_SPLIT, d_ff)
    w2 = B_w2.reshape(W2_SPLIT, d_ff // W2_SPLIT, d_model)

    hbm = pl.BlockSpec(memory_space=pltpu.HBM)
    return pl.pallas_call(
        functools.partial(_kernel, window=window),
        in_specs=[hbm] * 8,
        out_specs=hbm,
        out_shape=jax.ShapeDtypeStruct(A_x.shape, A_x.dtype),
        scratch_shapes=[
            pltpu.VMEM(A_x.shape, A_x.dtype),
            pltpu.VMEM((HQ * DH // WQ_COLS,) + wq.shape[:2] + (WQ_COLS,), bf16),
            pltpu.VMEM(w1.shape, bf16),
            pltpu.VMEM(w3.shape, bf16),
            pltpu.VMEM(w2.shape, bf16),
            pltpu.VMEM((WO_SPLIT, HQ // WO_SPLIT, DH, d_model), bf16),
            pltpu.VMEM((4 * (window // KV_COLS), DH, KV_COLS), bf16),
            pltpu.VMEM((HQ * DH // WQ_COLS, M, WQ_COLS), f32),
            pltpu.VMEM((HQ, M, DH), f32),
            pltpu.VMEM((HQ, M, DH), f32),
            pltpu.SemaphoreType.DMA(()),
        ],
        compiler_params=pltpu.CompilerParams(vmem_limit_bytes=64 * 1024 * 1024),
    )(A_x, kt, vt, wq, wo, w1, w3, w2)
```

```python
import functools

import jax
import jax.numpy as jnp
from jax import lax
import jax.experimental.pallas as pl
import jax.experimental.pallas.tpu as pltpu

HQ, DH = 32, 192
EPS = 1e-5
M = 8
RG = 8

LOOKAHEAD = 8
KV_COLS, KV_COPY_COLS = 1024, 512
WQ_COLS = 1024
KV_SPLIT, WQ_SPLIT, W13_SPLIT, W2_SPLIT, WO_SPLIT = 4, 10, 4, 3, 8


def _stream(x_hbm, k_hbm, v_hbm, wq_hbm, wo_hbm, w1_hbm, w3_hbm, w2_hbm, out_hbm,
            x_v, wq_v, w1_v, w3_v, w2_v, wo_v, kv_v, qf_v, q_v, o_v, io_sem, sems, *, window):
    f32, bf16 = jnp.float32, jnp.bfloat16
    ds = pl.ds
    n_heads, sk = k_hbm.shape[0], k_hbm.shape[-1]
    d_model, d_ff = x_v.shape[-1], w1_v.shape[-1]
    ng = window // KV_COLS
    per_head = 2 * ng
    groups = n_heads // WO_SPLIT

    def batches(copies, n):
        return [copies[i:i + n] for i in range(0, len(copies), n)]

    def same_place(src, dst, *idx):
        return src.at[idx], dst.at[idx]

    pre, q_ready = [], {}
    for g in range(wq_v.shape[0]):
        pre += batches([(wq_hbm.at[ds(a, 2), ds(r, RG), ds(g * WQ_COLS, WQ_COLS)], wq_v.at[g, ds(a, 2), ds(r, RG)])
                        for r in range(0, wq_v.shape[2], RG) for a in range(0, WQ_SPLIT, 2)], WQ_SPLIT)
        q_ready[len(pre) - 1] = g
    ffn = [same_place(src, dst, ds(a, 2), ds(r, RG))
           for r in range(0, w1_v.shape[1], RG) for a in range(0, W13_SPLIT, 2)
           for src, dst in ((w1_hbm, w1_v), (w3_hbm, w3_v))]
    half = w2_v.shape[1] // 2
    ffn += [same_place(w2_hbm, w2_v, slice(None), ds(r + off, RG)) for r in range(0, half, RG) for off in (0, half)]
    pre += batches(ffn, 12)

    post, wo_ready = [], {}
    for j in range(groups):
        for lo, hi in ((0, 128), (128, DH)):
            post += batches([(wo_hbm.at[ds(a, 4), ds(j * DH + r, RG)], wo_v.at[ds(a, 4), j, ds(r, RG)])
                             for r in range(lo, hi, RG) for a in range(0, WO_SPLIT, 4)], 16)
            wo_ready[len(post) - 1] = (j, lo, hi)
    assert per_head == LOOKAHEAD and len(pre) >= LOOKAHEAD and len(post) >= LOOKAHEAD

    def sem(n):
        return sems.at[n % LOOKAHEAD]

    def start(copies, n):
        for i, (src, dst) in enumerate(copies):
            pltpu.make_async_copy(src, dst, sem(n)).start(priority=i % 2)

    def wait(copies, n):
        for src, dst in copies:
            pltpu.make_async_copy(src, dst, sem(n)).wait()

    def kv_slot(h, r):
        return (h % 2) * per_head + r

    def start_kv(h, r):
        src = k_hbm if r < ng else v_hbm
        col = sk - window + (r % ng) * KV_COLS
        start([(src.at[h, :, ds(i, RG), ds(col + c, KV_COPY_COLS)],
                kv_v.at[kv_slot(h, r), :, ds(i, RG), ds(c, KV_COPY_COLS)])
               for c in range(0, KV_COLS, KV_COPY_COLS) for i in range(0, DH // KV_SPLIT, RG)], len(pre) + r)

    start(pre[0], 0)
    x_copy = pltpu.make_async_copy(x_hbm, x_v, io_sem)
    x_copy.start()
    for n in range(1, LOOKAHEAD):
        start(pre[n], n)
    x_copy.wait()
    x = x_v[0].astype(f32)
    xc = x - jnp.mean(x, axis=-1, keepdims=True)
    var = jnp.mean(xc * xc, axis=-1, keepdims=True)
    xn = jnp.broadcast_to(xc / jnp.sqrt(var + EPS), (M, d_model)).astype(bf16)

    for n, copies in enumerate(pre):
        wait(copies, n)
        if n + LOOKAHEAD < len(pre):
            start(pre[n + LOOKAHEAD], n + LOOKAHEAD)
        else:
            start_kv(0, n + LOOKAHEAD - len(pre))
        if n in q_ready:
            g = q_ready[n]
            qf_v[g] = jnp.dot(xn, wq_v[g].reshape(d_model, WQ_COLS), preferred_element_type=f32)
    gate = jnp.dot(xn, w1_v[...].reshape(d_model, d_ff), preferred_element_type=f32)
    up = jnp.dot(xn, w3_v[...].reshape(d_model, d_ff), preferred_element_type=f32)
    hidden = (gate * jax.nn.sigmoid(gate) * up).astype(bf16)
    ffn_out = jnp.dot(hidden, w2_v[...].reshape(d_ff, d_model), preferred_element_type=f32)
    ffn_gate = ffn_out * jax.nn.sigmoid(ffn_out)

    for h in range(n_heads):
        lo, hi = h * DH, (h + 1) * DH
        g0, g1 = lo // WQ_COLS, (hi - 1) // WQ_COLS
        if g0 == g1:
            q_v[h] = qf_v[g0, :, lo - g0 * WQ_COLS:hi - g0 * WQ_COLS]
        else:
            q_v[h] = jnp.concatenate([qf_v[g0, :, lo - g0 * WQ_COLS:], qf_v[g1, :, :hi - g1 * WQ_COLS]], axis=-1)

    scale = DH ** -0.5

    def head(h, carry):
        def next_tile(r):
            tile = kv_v.at[kv_slot(h, r)]
            wait([(tile, tile)], len(pre) + r)
            pl.when(h + 1 < n_heads)(lambda: start_kv(h + 1, r))
            pl.when(h + 1 == n_heads)(lambda: start(post[r], len(pre) + r))
            return tile[...].reshape(DH, KV_COLS)

        q = q_v[h].astype(bf16)
        s = [jnp.dot(q, next_tile(r), preferred_element_type=f32) * scale for r in range(ng)]
        m = jnp.max(functools.reduce(jnp.maximum, s), axis=-1, keepdims=True)
        p = [jnp.exp(si - m) for si in s]
        denom = jnp.sum(functools.reduce(jnp.add, p), axis=-1, keepdims=True)
        acc = jnp.zeros((M, DH), f32)
        for r in range(ng):
            acc = acc + lax.dot_general(p[r].astype(bf16), next_tile(ng + r), (((1,), (1,)), ((), ())),
                                        preferred_element_type=f32)
        o_v[h] = acc / denom
        return carry
    lax.fori_loop(0, n_heads, head, 0)

    y = jnp.zeros((M, d_model), f32)
    for n, copies in enumerate(post):
        if n in wo_ready:
            j, lo, hi = wo_ready[n]
            o = jnp.concatenate([o_v[a * groups + j, :, lo:hi] for a in range(WO_SPLIT)], axis=-1).astype(bf16)
        wait(copies, len(pre) + n)
        if n + LOOKAHEAD < len(post):
            start(post[n + LOOKAHEAD], len(pre) + n + LOOKAHEAD)
        if n in wo_ready:
            w = wo_v[:, j, lo:hi, :].reshape(WO_SPLIT * (hi - lo), d_model)
            y = y + jnp.dot(o, w, preferred_element_type=f32)

    x_v[0] = (x + y[0:1] * ffn_gate[0:1]).astype(x_v.dtype)
    pltpu.make_async_copy(x_v, out_hbm, io_sem).start()


def _kernel(*refs, window):
    out_hbm, x_v, io_sem = refs[8], refs[9], refs[-1]
    pl.run_scoped(functools.partial(_stream, *refs, window=window), pltpu.SemaphoreType.DMA((LOOKAHEAD,)))
    pltpu.make_async_copy(x_v, out_hbm, io_sem).wait()


@jax.jit
def pallas_recurrent_scan__sliding_block_cached__glu_gated_swiglu__decode_kernel(
    A_x: jax.Array,
    A_k_cache: jax.Array,
    A_v_cache: jax.Array,
    A_wq: jax.Array,
    A_wo: jax.Array,
    B_x: jax.Array,
    B_w1: jax.Array,
    B_w3: jax.Array,
    B_w2: jax.Array,
):
    del B_x
    d_model = A_x.shape[-1]
    _, hkv, sk, dh = A_k_cache.shape
    d_ff = B_w1.shape[1]
    window = min(4096, max(256, sk // 4))
    assert A_x.shape[:2] == (1, 1) and (hkv, dh) == (HQ, DH) and window % KV_COLS == 0
    bf16, f32 = jnp.bfloat16, jnp.float32

    kt = jnp.swapaxes(A_k_cache, 2, 3).reshape(hkv, KV_SPLIT, dh // KV_SPLIT, sk)
    vt = jnp.swapaxes(A_v_cache, 2, 3).reshape(hkv, KV_SPLIT, dh // KV_SPLIT, sk)
    wq = A_wq.reshape(WQ_SPLIT, d_model // WQ_SPLIT, HQ * DH)
    wo = A_wo.reshape(WO_SPLIT, HQ * DH // WO_SPLIT, d_model)
    w1 = B_w1.reshape(W13_SPLIT, d_model // W13_SPLIT, d_ff)
    w3 = B_w3.reshape(W13_SPLIT, d_model // W13_SPLIT, d_ff)
    w2 = B_w2.reshape(W2_SPLIT, d_ff // W2_SPLIT, d_model)

    hbm = pl.BlockSpec(memory_space=pltpu.HBM)
    return pl.pallas_call(
        functools.partial(_kernel, window=window),
        in_specs=[hbm] * 8,
        out_specs=hbm,
        out_shape=jax.ShapeDtypeStruct(A_x.shape, A_x.dtype),
        scratch_shapes=[
            pltpu.VMEM(A_x.shape, A_x.dtype),
            pltpu.VMEM((HQ * DH // WQ_COLS,) + wq.shape[:2] + (WQ_COLS,), bf16),
            pltpu.VMEM(w1.shape, bf16),
            pltpu.VMEM(w3.shape, bf16),
            pltpu.VMEM(w2.shape, bf16),
            pltpu.VMEM((WO_SPLIT, HQ // WO_SPLIT, DH, d_model), bf16),
            pltpu.VMEM((4 * (window // KV_COLS),) + kt.shape[1:3] + (KV_COLS,), bf16),
            pltpu.VMEM((HQ * DH // WQ_COLS, M, WQ_COLS), f32),
            pltpu.VMEM((HQ, M, DH), f32),
            pltpu.VMEM((HQ, M, DH), f32),
            pltpu.SemaphoreType.DMA(()),
        ],
        compiler_params=pltpu.CompilerParams(vmem_limit_bytes=64 * 1024 * 1024),
    )(A_x, kt, vt, wq, wo, w1, w3, w2)
```
